```python
import jax
import jax.numpy as jnp

def _softmax(x, axis=-1):
    return jax.nn.softmax(x, axis=axis)

def _gelu(x):
    return jax.nn.gelu(x, approximate=True)

def _silu(x):
    return jax.nn.silu(x)

def _sigmoid(x):
    return jax.nn.sigmoid(x)

def _layernorm(x, axis=-1, eps=1e-05):
    m = jnp.mean(x, axis=axis, keepdims=True)
    v = jnp.var(x, axis=axis, keepdims=True)
    return (x - m) / jnp.sqrt(v + eps)

def _scatter_add(tgt, idx, src, axis=0):
    return tgt.at[idx].add(src)

def _segment_sum(src, seg, n):
    return jax.ops.segment_sum(src, seg, n)

class _Rng:

    def __init__(self, key):
        self._k = key

    def _next(self):
        self._k, sub = jax.random.split(self._k)
        return sub

    def normal(self, shape):
        return jax.random.normal(self._next(), shape, dtype=jnp.bfloat16)

    def randint(self, lo, hi, shape):
        return jax.random.randint(self._next(), shape, lo, hi, dtype=jnp.int32)

    def uniform(self, shape, lo=0.0, hi=1.0):
        return jax.random.uniform(self._next(), shape, jnp.bfloat16, lo, hi)

    def permutation(self, n):
        return jax.random.permutation(self._next(), n)
kernel_name = 'adaLN_cond__memory_aug_recurrent_mem_tr__moe_arch_mod__prompt'

def setup_inputs():
    _rng = _Rng(jax.random.key(int.from_bytes(__import__("os").urandom(4), "little")))
    _w = lambda a: (lambda t: t.astype(jnp.bfloat16) if jnp.issubdtype(t.dtype, jnp.floating) else t)(jnp.asarray(a))

    def _A_setup():
        B, S, Dm = (1, 2048, 1024)
        H, Dh = (32, 128)
        M, seg = (8, 32)
        seg = min(seg, S)
        S = S // seg * seg
        return {'x': _w((lambda *s: _rng.normal(s) * 0.05)(B, S, Dm)), 'mem0': _w((lambda *s: _rng.normal(s) * 0.05)(B, M, Dm)), 'Wq': _w((lambda *s: _rng.normal(s) * 0.05)(Dm, H, Dh) * Dm ** (-0.5)), 'Wk': _w((lambda *s: _rng.normal(s) * 0.05)(Dm, H, Dh) * Dm ** (-0.5)), 'Wv': _w((lambda *s: _rng.normal(s) * 0.05)(Dm, H, Dh) * Dm ** (-0.5)), 'Wo': _w((lambda *s: _rng.normal(s) * 0.05)(H, Dh, Dm) * (H * Dh) ** (-0.5)), 'seg_len': seg}
    _A_in = _A_setup()

    def _B_setup():
        B, S, D, F, C = (1, 2048, 1024, 3584, 2)
        return {'x': _w((lambda *s: _rng.normal(s) * 0.05)(B, S, D)), 'w_r': _w((lambda *s: _rng.normal(s) * 0.05)(D)), 'w_gate': _w((lambda *s: _rng.normal(s) * 0.05)(D, F)), 'w_up': _w((lambda *s: _rng.normal(s) * 0.05)(D, F)), 'w_down': _w((lambda *s: _rng.normal(s) * 0.05)(F, D))}
    _B_in = _B_setup()
    return {'A_x': _A_in['x'], 'A_mem0': _A_in['mem0'], 'A_Wq': _A_in['Wq'], 'A_Wk': _A_in['Wk'], 'A_Wv': _A_in['Wv'], 'A_Wo': _A_in['Wo'], 'A_seg_len': _A_in['seg_len'], 'B_x': _B_in['x'], 'B_w_r': _B_in['w_r'], 'B_w_gate': _B_in['w_gate'], 'B_w_up': _B_in['w_up'], 'B_w_down': _B_in['w_down'], 'c': _w((lambda *s: _rng.normal(s) * 0.05)(1, 1024)), 'w_mod': _w((lambda *s: _rng.normal(s) * 0.05)(1024, 6 * 1024) * 1024 ** (-0.5))}

def reference(A_x, A_mem0, A_Wq, A_Wk, A_Wv, A_Wo, A_seg_len, B_x, B_w_r, B_w_gate, B_w_up, B_w_down, c, w_mod):

    def _A_ref(x, mem0, Wq, Wk, Wv, Wo, seg_len):
        B, S, Dm = x.shape
        H, Dh = (Wq.shape[1], Wq.shape[2])
        M = mem0.shape[1]
        scale = Dh ** (-0.5)
        n_seg = S // seg_len
        L = M + seg_len
        idx = jnp.arange(L)
        mask = (idx[:, None] < M) | (idx[:, None] >= idx[None, :])
        mem = mem0
        outs = []
        for s in range(n_seg):
            xs = x[:, s * seg_len:(s + 1) * seg_len, :].copy()
            h = jnp.concatenate([mem, xs], axis=1)
            q = jnp.einsum('btd,dhe->bhte', h, Wq)
            k = jnp.einsum('btd,dhe->bhte', h, Wk)
            v = jnp.einsum('btd,dhe->bhte', h, Wv)
            scores = jnp.einsum('bhqe,bhke->bhqk', q, k) * scale
            scores = jnp.where(mask[None, None], scores, -1000000000.0)
            p = _softmax(scores, axis=-1)
            o = jnp.einsum('bhqk,bhke->bhqe', p, v)
            o = jnp.einsum('bhte,hed->btd', o, Wo)
            mem = o[:, :M, :].copy()
            outs.append(o[:, M:, :])
        return jnp.concatenate(outs, axis=1)

    def _B_ref(x, w_r, w_gate, w_up, w_down):
        B, S, D = x.shape
        C = 2
        r = x @ w_r
        idx = jnp.argsort(-r, axis=-1)[:, :C]
        idx_e = jnp.repeat(idx.reshape(B, C, 1), D, axis=2)
        x_sel = jnp.take_along_axis(x, idx_e, axis=1)
        g = _silu(x_sel @ w_gate)
        u = x_sel @ w_up
        y = g * u @ w_down
        r_sel = _sigmoid(jnp.take_along_axis(r, idx, axis=1))
        y = y * r_sel.reshape(B, C, 1)
        b_off = (jnp.arange(B) * S).reshape(B, 1)
        flat_idx = (idx + b_off).reshape(B * C)
        zero = (x * 0.0).reshape(B * S, D)
        upd = _scatter_add(zero, flat_idx, y.reshape(B * C, D), axis=0)
        return x + upd.reshape(B, S, D)
    x = A_x
    mod = (_silu(c) @ w_mod).reshape(c.shape[0], 6, 1, -1)
    sa, ca, ga, sb, cb, gb = (mod[:, 0].copy(), mod[:, 1].copy(), mod[:, 2].copy(), mod[:, 3].copy(), mod[:, 4].copy(), mod[:, 5].copy())
    h = _layernorm(x, axis=-1) * (1 + ca) + sa
    x = x + ga * _A_ref(h, A_mem0, A_Wq, A_Wk, A_Wv, A_Wo, A_seg_len)
    h = _layernorm(x, axis=-1) * (1 + cb) + sb
    x = x + gb * _B_ref(h, B_w_r, B_w_gate, B_w_up, B_w_down)
    return x
```

```python
import functools

import jax
import jax.numpy as jnp
from jax import lax
import jax.experimental.pallas as pl
import jax.experimental.pallas.tpu as pltpu

F32 = jnp.float32
BF16 = jnp.bfloat16
U32 = jnp.uint32

S, D = 2048, 1024
NH, DH = 32, 128
MM, SEG = 8, 32
L = MM + SEG
LP = 48
NSEG = S // SEG
FF = 3584
KT = D // 128
EPS = 1e-05


def _ln(x):
    m = jnp.mean(x, axis=-1, keepdims=True)
    xc = x - m
    v = jnp.mean(xc * xc, axis=-1, keepdims=True)
    return xc * lax.rsqrt(v + EPS)


def _rb(x):
    return x.astype(BF16).astype(F32)


def _w(ref32, j):
    return pltpu.bitcast(ref32[j], BF16)


def _panel_dot(lhs, ref32, panels):
    return [jnp.dot(lhs, _w(ref32, j), preferred_element_type=F32) for j in panels]


def _kernel(x_hbm, mem0_ref, wq_hbm, wk_hbm, wv_hbm, wo_hbm, wr_ref, wg_hbm, wu_hbm,
            wd_hbm, c_ref, wmod_hbm, out_hbm,
            stg0, stg1, wqkv, wo, wg, wu, wd, wmod, xb, x1b, ob, modb, memb, hxb, oxb,
            obuf, rb, sem_st, sem_w, sem_o, sem_p):
    def panel_copies(src, dst, panels, sem, col0=0):
        return [pltpu.make_async_copy(src.at[:, pl.ds((col0 + j) * 128, 128)],
                                      dst.at[col0 + j], sem) for j in range(panels)]

    cp_moda = panel_copies(wmod_hbm, wmod, 16, sem_w.at[0])
    cp_x = pltpu.make_async_copy(x_hbm, xb, sem_w.at[1])
    cp_q = pltpu.make_async_copy(wq_hbm, stg0, sem_st.at[0])
    cp_k = pltpu.make_async_copy(wk_hbm, stg1, sem_st.at[1])
    cp_v = pltpu.make_async_copy(wv_hbm, stg0, sem_st.at[0])
    cp_wo = panel_copies(wo_hbm, wo, 8, sem_w.at[2])
    cp_modb = panel_copies(wmod_hbm, wmod, 32, sem_w.at[3], col0=16)
    cp_g = panel_copies(wg_hbm, wg, FF // 128, sem_w.at[4])
    cp_u = panel_copies(wu_hbm, wu, FF // 128, sem_w.at[5])
    cp_d = panel_copies(wd_hbm, wd, 8, sem_w.at[6])

    for cp in cp_moda:
        cp.start()
    cp_q.start()
    cp_k.start()
    cp_x.start()

    cv = c_ref[...].astype(F32)
    sc = jnp.broadcast_to(cv * jax.nn.sigmoid(cv), (8, D))
    wmod32 = wmod.bitcast(U32)

    def mod_part(lo, hi):
        for j in range(lo, hi):
            modb[:, (j // 8) * D + (j % 8) * 128:(j // 8) * D + (j % 8 + 1) * 128] = _rb(
                jnp.dot(sc, _w(wmod32, j), preferred_element_type=F32))

    for cp in cp_moda:
        cp.wait()
    mod_part(0, 16)

    def relayout(stg, t):
        s32 = stg.bitcast(U32)

        def body(i, carry):
            r = pl.ds(pl.multiple_of(i * 8, 8), 8)
            for p in range(NH // 2):
                a = s32[i, pl.ds(p, 8, stride=32), :]
                b = s32[i, pl.ds(16 + p, 8, stride=32), :]
                wqkv[t * NH + 2 * p, r, :] = (a & 0xFFFF) | (b << 16)
                wqkv[t * NH + 2 * p + 1, r, :] = (a >> 16) | ((b >> 16) << 16)
            return carry

        lax.fori_loop(0, D // 16, body, 0)

    cp_q.wait()
    relayout(stg0, 0)
    cp_v.start()
    for cp in cp_wo:
        cp.start()
    for cp in cp_modb:
        cp.start()
    for cp in cp_g + cp_u + cp_d:
        cp.start()
    cp_k.wait()
    relayout(stg1, 1)
    cp_x.wait()

    def sa_ca():
        return modb[0:1, 0:D], modb[0:1, D:2 * D]

    def make_hx(s):
        r = pl.ds(pl.multiple_of(s * SEG, SEG), SEG)
        sa, ca = sa_ca()
        hxb[...] = _ln(xb[r, :].astype(F32)) * (1.0 + ca) + sa

    memb[...] = mem0_ref[...].astype(F32)
    make_hx(0)
    oxb[...] = jnp.zeros(oxb.shape, F32)

    cp_v.wait()
    relayout(stg0, 2)
    for cp in cp_wo:
        cp.wait()
    for cp in cp_modb:
        cp.wait()
    mod_part(16, 48)

    wo32 = wo.bitcast(U32)
    wr = wr_ref[...].astype(F32)

    row = lax.broadcasted_iota(jnp.int32, (L, LP), 0)
    col = lax.broadcasted_iota(jnp.int32, (L, LP), 1)
    amask = ((row < MM) & (col < L)) | (row >= col)
    scale = float(DH) ** (-0.5)

    def post(s):
        r = pl.ds(pl.multiple_of(s * SEG, SEG), SEG)
        ga = modb[0:1, 2 * D:3 * D]
        sb = modb[0:1, 3 * D:4 * D]
        cb = modb[0:1, 4 * D:5 * D]
        gb = modb[0:1, 5 * D:6 * D]
        x1 = (xb[r, :].astype(F32) + ga * _rb(oxb[...])).astype(BF16)
        x1b[r, :] = x1
        x1 = x1.astype(F32)
        h2 = _ln(x1) * (1.0 + cb) + sb
        ob[r, :] = (x1 + gb * h2).astype(BF16)
        rr = jnp.sum(h2 * wr, axis=-1, keepdims=True)
        rb[r, :] = jnp.broadcast_to(rr, (SEG, 128))

    def out_copy(s):
        r = pl.ds(pl.multiple_of(s * SEG, SEG), SEG)
        return pltpu.make_async_copy(ob.at[r, :], out_hbm.at[r, :], sem_o)

    def step(s, carry):
        post(jnp.maximum(s - 1, 0))
        hh = jnp.concatenate([memb[...], hxb[...]], axis=0)
        zpad = jnp.zeros((LP - L, DH), F32)
        for h in range(NH):
            q, k, v = _panel_dot(hh, wqkv, (h, NH + h, 2 * NH + h))
            kb = jnp.concatenate([k, zpad], axis=0).astype(BF16)
            vb = jnp.concatenate([v, zpad], axis=0).astype(BF16)
            sc_ = lax.dot_general(q, kb, (((1,), (1,)), ((), ())),
                                  preferred_element_type=F32)
            sc_ = jnp.where(amask, sc_ * scale, -1000000000.0)
            e = jnp.exp(sc_ - jnp.max(sc_, axis=-1, keepdims=True))
            p = e / jnp.sum(e, axis=-1, keepdims=True)
            obuf[:, h * DH:(h + 1) * DH] = jnp.dot(p, vb, preferred_element_type=F32)
        oo = obuf[...]
        for n in range(KT):
            y = jnp.dot(oo, _w(wo32, n), preferred_element_type=F32)
            memb[:, n * 128:(n + 1) * 128] = y[0:MM]
            oxb[:, n * 128:(n + 1) * 128] = y[MM:L]
        make_hx(jnp.minimum(s + 1, NSEG - 1))

        @pl.when(s > 0)
        def _():
            out_copy(s - 1).start()
        return carry

    lax.fori_loop(0, NSEG, step, 0)
    post(NSEG - 1)
    out_copy(NSEG - 1).start()

    rv = rb[...]
    ridx = lax.broadcasted_iota(jnp.int32, (S, 128), 0)
    m1 = jnp.max(rv, axis=0, keepdims=True)
    i1v = jnp.min(jnp.where(rv == m1, ridx, S), axis=0, keepdims=True)
    rv2 = jnp.where(ridx == i1v, -jnp.inf, rv)
    m2 = jnp.max(rv2, axis=0, keepdims=True)
    i2v = jnp.min(jnp.where((rv2 == m2) & (ridx != i1v), ridx, S), axis=0, keepdims=True)
    idx = (jnp.min(i1v), jnp.min(i2v))
    rsel = (m1[:, 0:1], m2[:, 0:1])

    sb = modb[0:1, 3 * D:4 * D]
    cb = modb[0:1, 4 * D:5 * D]
    gb = modb[0:1, 5 * D:6 * D]
    brow = lax.broadcasted_iota(jnp.int32, (16, D), 0)
    blks, x1s, h2s, sel = [], [], [], []
    for j in range(2):
        b = pl.ds(pl.multiple_of((idx[j] // 16) * 16, 16), 16)
        x1 = x1b[b, :].astype(F32)
        h2 = _ln(x1) * (1.0 + cb) + sb
        blks.append(b)
        x1s.append(x1)
        h2s.append(h2)
        sel.append(jnp.sum(jnp.where(brow == idx[j] % 16, h2, 0.0), axis=0, keepdims=True))
    xs = jnp.concatenate(sel + [jnp.zeros((6, D), F32)], axis=0)

    for cp in cp_g + cp_u:
        cp.wait()
    wg32, wu32, wd32 = wg.bitcast(U32), wu.bitcast(U32), wd.bitcast(U32)
    npf = FF // 128
    gs = _panel_dot(xs, wg32, range(npf))
    us = _panel_dot(xs, wu32, range(npf))
    act = jnp.concatenate([g * jax.nn.sigmoid(g) * u for g, u in zip(gs, us)], axis=1)
    for cp in cp_d:
        cp.wait()
    y = jnp.concatenate(_panel_dot(act, wd32, range(KT)), axis=1)
    upd = [y[j:j + 1] * jax.nn.sigmoid(rsel[j]) for j in range(2)]

    pltpu.make_async_copy(ob, out_hbm, sem_o).wait()
    for j in range(2):
        base = (idx[j] // 16) * 16
        u = (jnp.where(brow + base == idx[0], upd[0], 0.0)
             + jnp.where(brow + base == idx[1], upd[1], 0.0))
        ob[blks[j], :] = (x1s[j] + gb * (h2s[j] + u)).astype(BF16)
        cp = pltpu.make_async_copy(ob.at[blks[j], :], out_hbm.at[blks[j], :], sem_p)
        cp.start()
        cp.wait()


@functools.partial(jax.jit, static_argnames=("A_seg_len",))
def pallas_adaLN_cond__memory_aug_recurrent_mem_tr__moe_arch_mod__prompt_kernel(
    A_x, A_mem0, A_Wq, A_Wk, A_Wv, A_Wo, A_seg_len, B_x, B_w_r, B_w_gate, B_w_up,
    B_w_down, c, w_mod,
):
    assert A_seg_len == SEG and A_x.shape == (1, S, D)
    assert A_Wq.shape == (D, NH, DH) and A_mem0.shape == (1, MM, D)
    del B_x
    hbm = pl.BlockSpec(memory_space=pl.ANY)
    vm = pl.BlockSpec(memory_space=pltpu.VMEM)
    npf = FF // 128
    out = pl.pallas_call(
        _kernel,
        out_shape=jax.ShapeDtypeStruct((S, D), BF16),
        in_specs=[hbm, vm, hbm, hbm, hbm, hbm, vm, hbm, hbm, hbm, vm, hbm],
        out_specs=hbm,
        scratch_shapes=[
            pltpu.VMEM((D // 16, 16 * NH, DH), BF16),
            pltpu.VMEM((D // 16, 16 * NH, DH), BF16),
            pltpu.VMEM((3 * NH, D // 2, 128), U32),
            pltpu.VMEM((KT, NH * DH, 128), BF16),
            pltpu.VMEM((npf, D, 128), BF16),
            pltpu.VMEM((npf, D, 128), BF16),
            pltpu.VMEM((KT, FF, 128), BF16),
            pltpu.VMEM((48, D, 128), BF16),
            pltpu.VMEM((S, D), BF16),
            pltpu.VMEM((S, D), BF16),
            pltpu.VMEM((S, D), BF16),
            pltpu.VMEM((8, 6 * D), F32),
            pltpu.VMEM((MM, D), F32),
            pltpu.VMEM((SEG, D), F32),
            pltpu.VMEM((SEG, D), F32),
            pltpu.VMEM((L, NH * DH), F32),
            pltpu.VMEM((S, 128), F32),
            pltpu.SemaphoreType.DMA((2,)),
            pltpu.SemaphoreType.DMA((7,)),
            pltpu.SemaphoreType.DMA,
            pltpu.SemaphoreType.DMA,
        ],
        compiler_params=pltpu.CompilerParams(vmem_limit_bytes=120 * 2**20),
    )(
        A_x.reshape(S, D), A_mem0.reshape(MM, D),
        A_Wq.reshape(D // 16, 16 * NH, DH), A_Wk.reshape(D // 16, 16 * NH, DH),
        A_Wv.reshape(D // 16, 16 * NH, DH), A_Wo.reshape(NH * DH, D),
        B_w_r.reshape(1, D), B_w_gate, B_w_up, B_w_down, c, w_mod,
    )
    return out.reshape(1, S, D)
```

```python
import functools

import jax
import jax.numpy as jnp
from jax import lax
import jax.experimental.pallas as pl
import jax.experimental.pallas.tpu as pltpu

F32 = jnp.float32
BF16 = jnp.bfloat16
U32 = jnp.uint32

S, D = 2048, 1024
NH, DH = 32, 128
MM, SEG = 8, 32
L = MM + SEG
LP = 48
NSEG = S // SEG
FF = 3584
KT = D // 128
EPS = 1e-05
LAG = 3
PR = 8
XE = 8 * SEG


def _ln(x):
    m = jnp.mean(x, axis=-1, keepdims=True)
    xc = x - m
    v = jnp.mean(xc * xc, axis=-1, keepdims=True)
    return xc * lax.rsqrt(v + EPS)


def _rb(x):
    return x.astype(BF16).astype(F32)


def _w(ref32, j):
    return pltpu.bitcast(ref32[j], BF16)


def _panel_dot(lhs, ref32, panels):
    return [jnp.dot(lhs, _w(ref32, j), preferred_element_type=F32) for j in panels]


def _kernel(x_hbm, x3_hbm, mem0_ref, wq_hbm, wk_hbm, wv_hbm, wo_hbm, wr_ref, wg_hbm, wu_hbm,
            wd_hbm, c_ref, wmod_hbm, out_hbm,
            stg0, stg1, stg2, wq, wk, wv, wo, wg, wu, wd, wmod, xb, xpre, hpre, x1b, ob, modb,
            memb, hxb, oxb, obuf, sem_st, sem_w, sem_o, sem_p):
    def panel_copies(src, dst, panels, sem, col0=0):
        return [pltpu.make_async_copy(src.at[:, pl.ds((col0 + j) * 128, 128)],
                                      dst.at[col0 + j], sem) for j in range(panels)]

    cp_moda = panel_copies(wmod_hbm, wmod, 16, sem_w.at[0])
    cp_x0 = pltpu.make_async_copy(x_hbm.at[0:XE], xb.at[0:XE], sem_w.at[1])
    cp_x1 = pltpu.make_async_copy(x_hbm.at[XE:S], xb.at[XE:S], sem_w.at[7])
    cp_xp = pltpu.make_async_copy(x3_hbm.at[:, 0:PR, :], xpre, sem_w.at[8])
    cp_q = pltpu.make_async_copy(wq_hbm, stg0, sem_st.at[0])
    cp_k = pltpu.make_async_copy(wk_hbm, stg1, sem_st.at[1])
    cp_v = pltpu.make_async_copy(wv_hbm, stg2, sem_st.at[2])
    cp_wo = panel_copies(wo_hbm, wo, 8, sem_w.at[2])

    def panel_copy(src, dst, j, sem):
        return pltpu.make_async_copy(
            src.at[:, pl.ds(pl.multiple_of(j * 128, 128), 128)], dst.at[j], sem)

    def modb_copy(j):
        return panel_copy(wmod_hbm, wmod, 16 + j, sem_w.at[3])

    for cp in cp_moda:
        cp.start()
    cp_xp.start()
    cp_q.start()

    cv = c_ref[...].astype(F32)
    sc = jnp.broadcast_to(cv * jax.nn.sigmoid(cv), (8, D))
    wmod32 = wmod.bitcast(U32)

    def mod_part(lo, hi):
        for j in range(lo, hi):
            modb[:, (j // 8) * D + (j % 8) * 128:(j // 8) * D + (j % 8 + 1) * 128] = _rb(
                jnp.dot(sc, _w(wmod32, j), preferred_element_type=F32))

    def sa_ca():
        return modb[0:1, 0:D], modb[0:1, D:2 * D]

    for cp in cp_moda:
        cp.wait()
    mod_part(0, 16)
    modb[:, 2 * D:6 * D] = jnp.zeros((8, 4 * D), F32)
    memb[...] = mem0_ref[...].astype(F32)
    oxb[...] = jnp.zeros(oxb.shape, F32)
    cp_xp.wait()

    def pre_ln(i, carry):
        sa, ca = sa_ca()
        xv = jnp.concatenate([xpre[i * 4 + j] for j in range(4)], axis=0).astype(F32)
        hpre[pl.ds(pl.multiple_of(i * 32, 32), 32), :] = _ln(xv) * (1.0 + ca) + sa
        return carry

    lax.fori_loop(0, NSEG // 4, pre_ln, 0)

    qpre = stg0.bitcast(F32)

    def relayout(stg, dst, half=None):
        s32 = stg.bitcast(U32)

        def body(i, carry):
            if half is not None:
                qpre[2 * i + half] = jnp.dot(
                    hpre[half * 256:(half + 1) * 256, :], _w(wq, i),
                    preferred_element_type=F32)
            if half == 1:
                modb_copy(i).start()
            for b in range(2):
                blk = 2 * i + b
                r = pl.ds(pl.multiple_of(blk * 8, 8), 8)
                for p in range(NH // 2):
                    a = s32[blk, pl.ds(p, 8, stride=32), :]
                    b_ = s32[blk, pl.ds(16 + p, 8, stride=32), :]
                    dst[2 * p, r, :] = (a & 0xFFFF) | (b_ << 16)
                    dst[2 * p + 1, r, :] = (a >> 16) | ((b_ >> 16) << 16)
            return carry

        lax.fori_loop(0, D // 32, body, 0, unroll=2)

    cp_q.wait()
    cp_k.start()
    relayout(stg0, wq)
    cp_v.start()
    cp_k.wait()
    cp_x0.start()
    for cp in cp_wo:
        cp.start()
    relayout(stg1, wk, 0)
    cp_v.wait()
    relayout(stg2, wv, 1)
    cp_x1.start()

    def make_hx(s):
        r = pl.ds(pl.multiple_of(s * SEG, SEG), SEG)
        sa, ca = sa_ca()
        hxb[...] = _ln(xb[r, :].astype(F32)) * (1.0 + ca) + sa

    cp_x0.wait()
    make_hx(0)
    for cp in cp_wo:
        cp.wait()

    wo32 = wo.bitcast(U32)
    wr = wr_ref[...].astype(F32)

    row = lax.broadcasted_iota(jnp.int32, (L, LP), 0)
    col = lax.broadcasted_iota(jnp.int32, (L, LP), 1)
    amask = ((row < MM) & (col < L)) | (row >= col)
    scale = float(DH) ** (-0.5)

    trow = lax.broadcasted_iota(jnp.int32, (8, 128), 0)

    def post(s, slot, top, valid=None):
        r = pl.ds(pl.multiple_of(s * SEG, SEG), SEG)
        ga = modb[0:1, 2 * D:3 * D]
        sb = modb[0:1, 3 * D:4 * D]
        cb = modb[0:1, 4 * D:5 * D]
        gb = modb[0:1, 5 * D:6 * D]
        x1 = (xb[r, :].astype(F32) + ga * _rb(oxb[slot])).astype(BF16)
        x1b[r, :] = x1
        x1 = x1.astype(F32)
        h2 = _ln(x1) * (1.0 + cb) + sb
        ob[r, :] = (x1 + gb * h2).astype(BF16)
        rr = jnp.broadcast_to(jnp.sum(h2 * wr, axis=-1, keepdims=True), (SEG, 128))
        if valid is not None:
            rr = jnp.where(valid, rr, -jnp.inf)
        v1, i1, v2, i2 = top
        for j in range(SEG // 8):
            val = rr[j * 8:(j + 1) * 8]
            ix = trow + (s * SEG + j * 8)
            g1, g2 = val > v1, val > v2
            v2 = jnp.where(g1, v1, jnp.where(g2, val, v2))
            i2 = jnp.where(g1, i1, jnp.where(g2, ix, i2))
            v1 = jnp.where(g1, val, v1)
            i1 = jnp.where(g1, ix, i1)
        return v1, i1, v2, i2

    def out_copy(s):
        r = pl.ds(pl.multiple_of(s * SEG, SEG), SEG)
        return pltpu.make_async_copy(ob.at[r, :], out_hbm.at[r, :], sem_o)

    def step(s, top):
        @pl.when(s == 2)
        def _():
            pltpu.make_async_copy(wmod.at[16:48], wmod.at[16:48], sem_w.at[3]).wait()
            mod_part(16, 48)

        @pl.when(s < FF // 128)
        def _():
            panel_copy(wg_hbm, wg, s, sem_w.at[4]).start()
            panel_copy(wu_hbm, wu, s, sem_w.at[5]).start()

        @pl.when(s < KT)
        def _():
            panel_copy(wd_hbm, wd, s, sem_w.at[6]).start()

        @pl.when(s == XE // SEG - 1)
        def _():
            cp_x1.wait()

        @pl.when(s > 2)
        def _():
            out_copy(s - 3).start()

        slot = s % 2
        top = post(jnp.maximum(s - 2, 0), slot, top, s >= 2)
        hq = jnp.concatenate([memb[...], hxb[PR:SEG, :]], axis=0)
        qrow = pl.ds(pl.multiple_of((s % 32) * PR, PR), PR)
        hh = jnp.concatenate([memb[...], hxb[...]], axis=0)
        zpad = jnp.zeros((LP - L, DH), F32)
        qs, ks, vs, ps = {}, {}, {}, {}

        def proj(h):
            q, = _panel_dot(hq, wq, (h,))
            k, = _panel_dot(hh, wk, (h,))
            v, = _panel_dot(hh, wv, (h,))
            qs[h] = jnp.concatenate([q[0:MM], qpre[2 * h + s // 32, qrow, :], q[MM:]], axis=0)
            ks[h] = jnp.concatenate([k, zpad], axis=0).astype(BF16)
            vs[h] = jnp.concatenate([v, zpad], axis=0).astype(BF16)

        def scores(h):
            sc_ = lax.dot_general(qs.pop(h), ks.pop(h), (((1,), (1,)), ((), ())),
                                  preferred_element_type=F32)
            sc_ = jnp.where(amask, sc_ * scale, -1000000000.0)
            e = jnp.exp(sc_ - jnp.max(sc_, axis=-1, keepdims=True))
            ps[h] = e / jnp.sum(e, axis=-1, keepdims=True)

        def pv(h):
            obuf[:, h * DH:(h + 1) * DH] = jnp.dot(ps.pop(h), vs.pop(h),
                                                   preferred_element_type=F32)

        HK = NH * DH // 2
        part = {}

        def oproj(n, half):
            w = pltpu.bitcast(wo32[n, half * (HK // 2):(half + 1) * (HK // 2), :], BF16)
            y = jnp.dot(obuf[:, half * HK:(half + 1) * HK], w, preferred_element_type=F32)
            if half == 0:
                part[n] = y
            else:
                y = y + part.pop(n)
                memb[:, n * 128:(n + 1) * 128] = y[0:MM]
                oxb[slot, :, n * 128:(n + 1) * 128] = y[MM:L]

        for i in range(NH + LAG):
            if i < NH:
                proj(i)
            else:
                if i == NH:
                    make_hx(jnp.minimum(s + 1, NSEG - 1))
                per = KT // LAG
                for n in range((i - NH) * per, KT if i == NH + LAG - 1 else (i - NH + 1) * per):
                    oproj(n, 0)
            if 0 <= i - 1 < NH:
                scores(i - 1)
            if 0 <= i - LAG < NH:
                pv(i - LAG)
        for n in range(KT):
            oproj(n, 1)

        return top

    ninf = jnp.full((8, 128), -jnp.inf, F32)
    top = lax.fori_loop(0, NSEG, step, (ninf, trow, ninf, trow + 8))
    out_copy(NSEG - 3).start()
    top = post(NSEG - 2, 0, top)
    out_copy(NSEG - 2).start()
    v1, i1, v2, i2 = post(NSEG - 1, 1, top)
    out_copy(NSEG - 1).start()

    m1 = jnp.max(v1, axis=0, keepdims=True)
    i1v = jnp.min(jnp.where(v1 == m1, i1, S), axis=0, keepdims=True)
    cv2 = jnp.where(i1 == i1v, v2, v1)
    ci2 = jnp.where(i1 == i1v, i2, i1)
    m2 = jnp.max(cv2, axis=0, keepdims=True)
    i2v = jnp.min(jnp.where(cv2 == m2, ci2, S), axis=0, keepdims=True)
    idx = (jnp.min(i1v), jnp.min(i2v))
    rsel = (m1[:, 0:1], m2[:, 0:1])

    sb = modb[0:1, 3 * D:4 * D]
    cb = modb[0:1, 4 * D:5 * D]
    gb = modb[0:1, 5 * D:6 * D]
    brow = lax.broadcasted_iota(jnp.int32, (16, D), 0)
    blks, x1s, h2s, sel = [], [], [], []
    for j in range(2):
        b = pl.ds(pl.multiple_of((idx[j] // 16) * 16, 16), 16)
        x1 = x1b[b, :].astype(F32)
        h2 = _ln(x1) * (1.0 + cb) + sb
        blks.append(b)
        x1s.append(x1)
        h2s.append(h2)
        sel.append(jnp.sum(jnp.where(brow == idx[j] % 16, h2, 0.0), axis=0, keepdims=True))
    xs = jnp.concatenate(sel + [jnp.zeros((6, D), F32)], axis=0)

    pltpu.make_async_copy(wg, wg, sem_w.at[4]).wait()
    pltpu.make_async_copy(wu, wu, sem_w.at[5]).wait()
    wg32, wu32, wd32 = wg.bitcast(U32), wu.bitcast(U32), wd.bitcast(U32)
    npf = FF // 128
    gs = _panel_dot(xs, wg32, range(npf))
    us = _panel_dot(xs, wu32, range(npf))
    act = jnp.concatenate([g * jax.nn.sigmoid(g) * u for g, u in zip(gs, us)], axis=1)
    pltpu.make_async_copy(wd, wd, sem_w.at[6]).wait()
    y = jnp.concatenate(_panel_dot(act, wd32, range(KT)), axis=1)
    upd = [y[j:j + 1] * jax.nn.sigmoid(rsel[j]) for j in range(2)]

    pltpu.make_async_copy(ob, out_hbm, sem_o).wait()
    for j in range(2):
        base = (idx[j] // 16) * 16
        u = (jnp.where(brow + base == idx[0], upd[0], 0.0)
             + jnp.where(brow + base == idx[1], upd[1], 0.0))
        ob[blks[j], :] = (x1s[j] + gb * (h2s[j] + u)).astype(BF16)
        cp = pltpu.make_async_copy(ob.at[blks[j], :], out_hbm.at[blks[j], :], sem_p)
        cp.start()
        cp.wait()


@functools.partial(jax.jit, static_argnames=("A_seg_len",))
def pallas_adaLN_cond__memory_aug_recurrent_mem_tr__moe_arch_mod__prompt_kernel(
    A_x, A_mem0, A_Wq, A_Wk, A_Wv, A_Wo, A_seg_len, B_x, B_w_r, B_w_gate, B_w_up,
    B_w_down, c, w_mod,
):
    assert A_seg_len == SEG and A_x.shape == (1, S, D)
    assert A_Wq.shape == (D, NH, DH) and A_mem0.shape == (1, MM, D)
    del B_x
    hbm = pl.BlockSpec(memory_space=pl.ANY)
    vm = pl.BlockSpec(memory_space=pltpu.VMEM)
    npf = FF // 128
    out = pl.pallas_call(
        _kernel,
        out_shape=jax.ShapeDtypeStruct((S, D), BF16),
        in_specs=[hbm, hbm, vm, hbm, hbm, hbm, hbm, vm, hbm, hbm, hbm, vm, hbm],
        out_specs=hbm,
        scratch_shapes=[
            pltpu.VMEM((D // 16, 16 * NH, DH), BF16),
            pltpu.VMEM((D // 16, 16 * NH, DH), BF16),
            pltpu.VMEM((D // 16, 16 * NH, DH), BF16),
            pltpu.VMEM((NH, D // 2, 128), U32),
            pltpu.VMEM((NH, D // 2, 128), U32),
            pltpu.VMEM((NH, D // 2, 128), U32),
            pltpu.VMEM((KT, NH * DH, 128), BF16),
            pltpu.VMEM((npf, D, 128), BF16),
            pltpu.VMEM((npf, D, 128), BF16),
            pltpu.VMEM((KT, FF, 128), BF16),
            pltpu.VMEM((48, D, 128), BF16),
            pltpu.VMEM((S, D), BF16),
            pltpu.VMEM((NSEG, PR, D), BF16),
            pltpu.VMEM((NSEG * PR, D), F32),
            pltpu.VMEM((S, D), BF16),
            pltpu.VMEM((S, D), BF16),
            pltpu.VMEM((8, 6 * D), F32),
            pltpu.VMEM((MM, D), F32),
            pltpu.VMEM((SEG, D), F32),
            pltpu.VMEM((2, SEG, D), F32),
            pltpu.VMEM((L, NH * DH), F32),
            pltpu.SemaphoreType.DMA((3,)),
            pltpu.SemaphoreType.DMA((9,)),
            pltpu.SemaphoreType.DMA,
            pltpu.SemaphoreType.DMA,
        ],
        compiler_params=pltpu.CompilerParams(vmem_limit_bytes=120 * 2**20),
    )(
        A_x.reshape(S, D), A_x.reshape(NSEG, SEG, D), A_mem0.reshape(MM, D),
        A_Wq.reshape(D // 16, 16 * NH, DH), A_Wk.reshape(D // 16, 16 * NH, DH),
        A_Wv.reshape(D // 16, 16 * NH, DH), A_Wo.reshape(NH * DH, D),
        B_w_r.reshape(1, D), B_w_gate, B_w_up, B_w_down, c, w_mod,
    )
    return out.reshape(1, S, D)
```

```python
import functools

import jax
import jax.numpy as jnp
from jax import lax
import jax.experimental.pallas as pl
import jax.experimental.pallas.tpu as pltpu

F32 = jnp.float32
BF16 = jnp.bfloat16
U32 = jnp.uint32

S, D = 2048, 1024
NH, DH = 32, 128
MM, SEG = 8, 32
L = MM + SEG
LP = 48
NSEG = S // SEG
FF = 3584
KT = D // 128
EPS = 1e-05
LAG = 3
PR = 8
XE = 8 * SEG


def _ln(x):
    m = jnp.mean(x, axis=-1, keepdims=True)
    xc = x - m
    v = jnp.mean(xc * xc, axis=-1, keepdims=True)
    return xc * lax.rsqrt(v + EPS)


def _rb(x):
    return x.astype(BF16).astype(F32)


def _w(ref32, j):
    return pltpu.bitcast(ref32[j], BF16)


def _panel_dot(lhs, ref32, panels):
    return [jnp.dot(lhs, _w(ref32, j), preferred_element_type=F32) for j in panels]


def _kernel(x_hbm, x3_hbm, mem0_ref, wq_hbm, wk_hbm, wv_hbm, wo_hbm, wr_ref, wg_hbm, wu_hbm,
            wd_hbm, c_ref, wmod_hbm, out_hbm,
            stg0, stg1, stg2, wq, wk, wv, wo, wg, wu, wd, wmod, xb, xpre, hpre, x1b, ob, modb,
            memb, hxb, oxb, obuf, sem_st, sem_w, sem_o, sem_p):
    def panel_copies(src, dst, panels, sem, col0=0):
        return [pltpu.make_async_copy(src.at[:, pl.ds((col0 + j) * 128, 128)],
                                      dst.at[col0 + j], sem) for j in range(panels)]

    cp_moda = panel_copies(wmod_hbm, wmod, 16, sem_w.at[0])
    cp_x0 = pltpu.make_async_copy(x_hbm.at[0:XE], xb.at[0:XE], sem_w.at[1])
    cp_x1 = pltpu.make_async_copy(x_hbm.at[XE:S], xb.at[XE:S], sem_w.at[7])
    cp_xp = pltpu.make_async_copy(x3_hbm.at[:, 0:PR, :], xpre, sem_w.at[8])
    cp_q = pltpu.make_async_copy(wq_hbm, stg0, sem_st.at[0])
    cp_k = pltpu.make_async_copy(wk_hbm, stg1, sem_st.at[1])
    cp_v = pltpu.make_async_copy(wv_hbm, stg2, sem_st.at[2])
    cp_wo = panel_copies(wo_hbm, wo, 8, sem_w.at[2])

    def panel_copy(src, dst, j, sem):
        return pltpu.make_async_copy(
            src.at[:, pl.ds(pl.multiple_of(j * 128, 128), 128)], dst.at[j], sem)

    def modb_copy(j):
        return panel_copy(wmod_hbm, wmod, 16 + j, sem_w.at[3])

    for cp in cp_moda:
        cp.start()
    cp_xp.start()
    cp_q.start()

    cv = c_ref[...].astype(F32)
    sc = jnp.broadcast_to(cv * jax.nn.sigmoid(cv), (8, D))
    wmod32 = wmod.bitcast(U32)

    def mod_part(lo, hi):
        for j in range(lo, hi):
            modb[:, (j // 8) * D + (j % 8) * 128:(j // 8) * D + (j % 8 + 1) * 128] = _rb(
                jnp.dot(sc, _w(wmod32, j), preferred_element_type=F32))

    def sa_ca():
        return modb[0:1, 0:D], modb[0:1, D:2 * D]

    for cp in cp_moda:
        cp.wait()
    mod_part(0, 16)
    modb[:, 2 * D:6 * D] = jnp.zeros((8, 4 * D), F32)
    memb[...] = mem0_ref[...].astype(F32)
    oxb[...] = jnp.zeros(oxb.shape, F32)
    cp_xp.wait()

    def pre_ln(i, carry):
        sa, ca = sa_ca()
        xv = jnp.concatenate([xpre[i * 4 + j] for j in range(4)], axis=0).astype(F32)
        hpre[pl.ds(pl.multiple_of(i * 32, 32), 32), :] = _ln(xv) * (1.0 + ca) + sa
        return carry

    lax.fori_loop(0, NSEG // 4, pre_ln, 0)

    qpre = stg0.bitcast(F32)

    def relayout(stg, dst, half=None):
        s32 = stg.bitcast(U32)

        def body(i, carry):
            if half is not None:
                qpre[2 * i + half] = jnp.dot(
                    hpre[half * 256:(half + 1) * 256, :], _w(wq, i),
                    preferred_element_type=F32)
            if half == 1:
                modb_copy(i).start()
            for b in range(2):
                blk = 2 * i + b
                r = pl.ds(pl.multiple_of(blk * 8, 8), 8)
                for p in range(NH // 2):
                    a = s32[blk, pl.ds(p, 8, stride=32), :]
                    b_ = s32[blk, pl.ds(16 + p, 8, stride=32), :]
                    dst[2 * p, r, :] = (a & 0xFFFF) | (b_ << 16)
                    dst[2 * p + 1, r, :] = (a >> 16) | ((b_ >> 16) << 16)
            return carry

        lax.fori_loop(0, D // 32, body, 0, unroll=2)

    cp_q.wait()
    cp_k.start()
    relayout(stg0, wq)
    cp_v.start()
    cp_k.wait()
    cp_x0.start()
    for cp in cp_wo:
        cp.start()
    relayout(stg1, wk, 0)
    cp_v.wait()
    relayout(stg2, wv, 1)
    cp_x1.start()

    def make_hx(s):
        r = pl.ds(pl.multiple_of(s * SEG, SEG), SEG)
        sa, ca = sa_ca()
        hxb[...] = _ln(xb[r, :].astype(F32)) * (1.0 + ca) + sa

    cp_x0.wait()
    make_hx(0)
    for cp in cp_wo:
        cp.wait()

    wo32 = wo.bitcast(U32)
    wr = wr_ref[...].astype(F32)

    row = lax.broadcasted_iota(jnp.int32, (L, LP), 0)
    col = lax.broadcasted_iota(jnp.int32, (L, LP), 1)
    amask = ((row < MM) & (col < L)) | (row >= col)
    scale = float(DH) ** (-0.5)

    trow = lax.broadcasted_iota(jnp.int32, (8, 128), 0)

    def post(s, slot, top, valid=None):
        r = pl.ds(pl.multiple_of(s * SEG, SEG), SEG)
        ga = modb[0:1, 2 * D:3 * D]
        sb = modb[0:1, 3 * D:4 * D]
        cb = modb[0:1, 4 * D:5 * D]
        gb = modb[0:1, 5 * D:6 * D]
        x1 = (xb[r, :].astype(F32) + ga * _rb(oxb[slot])).astype(BF16)
        x1b[r, :] = x1
        x1 = x1.astype(F32)
        h2 = _ln(x1) * (1.0 + cb) + sb
        ob[r, :] = (x1 + gb * h2).astype(BF16)
        rr = jnp.broadcast_to(jnp.sum(h2 * wr, axis=-1, keepdims=True), (SEG, 128))
        if valid is not None:
            rr = jnp.where(valid, rr, -jnp.inf)
        v1, i1, v2, i2 = top
        for j in range(SEG // 8):
            val = rr[j * 8:(j + 1) * 8]
            ix = trow + (s * SEG + j * 8)
            g1, g2 = val > v1, val > v2
            v2 = jnp.where(g1, v1, jnp.where(g2, val, v2))
            i2 = jnp.where(g1, i1, jnp.where(g2, ix, i2))
            v1 = jnp.where(g1, val, v1)
            i1 = jnp.where(g1, ix, i1)
        return v1, i1, v2, i2

    def out_copy(s):
        r = pl.ds(pl.multiple_of(s * SEG, SEG), SEG)
        return pltpu.make_async_copy(ob.at[r, :], out_hbm.at[r, :], sem_o)

    def step2(s2, top):
        s0 = 2 * s2

        @pl.when(s2 == 1)
        def _():
            pltpu.make_async_copy(wmod.at[16:48], wmod.at[16:48], sem_w.at[3]).wait()
            mod_part(16, 48)

        @pl.when(s2 < FF // 256)
        def _():
            for j in range(2):
                panel_copy(wg_hbm, wg, s0 + j, sem_w.at[4]).start()
                panel_copy(wu_hbm, wu, s0 + j, sem_w.at[5]).start()

        @pl.when(s2 < KT // 2)
        def _():
            for j in range(2):
                panel_copy(wd_hbm, wd, s0 + j, sem_w.at[6]).start()

        @pl.when(s2 == (XE // SEG - 1) // 2)
        def _():
            cp_x1.wait()

        @pl.when(s2 >= 2)
        def _():
            out_copy(s0 - 4).start()
            out_copy(s0 - 3).start()

        top = step(s0, 0, top)
        return step(s0 + 1, 1, top)

    def step(s, slot, top):
        top = post(jnp.maximum(s - 2, 0), slot, top, s >= 2)
        hq = jnp.concatenate([memb[...], hxb[PR:SEG, :]], axis=0)
        qrow = pl.ds(pl.multiple_of((s % 32) * PR, PR), PR)
        hh = jnp.concatenate([memb[...], hxb[...]], axis=0)
        zpad = jnp.zeros((LP - L, DH), F32)
        qs, ks, vs, ps = {}, {}, {}, {}

        def proj(h):
            q, = _panel_dot(hq, wq, (h,))
            k, = _panel_dot(hh, wk, (h,))
            v, = _panel_dot(hh, wv, (h,))
            qs[h] = jnp.concatenate([q[0:MM], qpre[2 * h + s // 32, qrow, :], q[MM:]], axis=0)
            ks[h] = jnp.concatenate([k, zpad], axis=0).astype(BF16)
            vs[h] = jnp.concatenate([v, zpad], axis=0).astype(BF16)

        def scores(h):
            sc_ = lax.dot_general(qs.pop(h), ks.pop(h), (((1,), (1,)), ((), ())),
                                  preferred_element_type=F32)
            sc_ = jnp.where(amask, sc_ * scale, -1000000000.0)
            e = jnp.exp(sc_ - jnp.max(sc_, axis=-1, keepdims=True))
            ps[h] = e / jnp.sum(e, axis=-1, keepdims=True)

        def pv(h):
            obuf[:, h * DH:(h + 1) * DH] = jnp.dot(ps.pop(h), vs.pop(h),
                                                   preferred_element_type=F32)

        HK = NH * DH // 2
        part = {}

        def oproj(n, half):
            w = pltpu.bitcast(wo32[n, half * (HK // 2):(half + 1) * (HK // 2), :], BF16)
            y = jnp.dot(obuf[:, half * HK:(half + 1) * HK], w, preferred_element_type=F32)
            if half == 0:
                part[n] = y
            else:
                y = y + part.pop(n)
                memb[:, n * 128:(n + 1) * 128] = y[0:MM]
                oxb[slot, :, n * 128:(n + 1) * 128] = y[MM:L]

        for i in range(NH + LAG):
            if i < NH:
                proj(i)
            else:
                if i == NH:
                    make_hx(jnp.minimum(s + 1, NSEG - 1))
                per = KT // LAG
                for n in range((i - NH) * per, KT if i == NH + LAG - 1 else (i - NH + 1) * per):
                    oproj(n, 0)
            if 0 <= i - 1 < NH:
                scores(i - 1)
            if 0 <= i - LAG < NH:
                pv(i - LAG)
        for n in range(KT):
            oproj(n, 1)

        return top

    ninf = jnp.full((8, 128), -jnp.inf, F32)
    top = lax.fori_loop(0, NSEG // 2, step2, (ninf, trow, ninf, trow + 8))
    out_copy(NSEG - 4).start()
    out_copy(NSEG - 3).start()
    top = post(NSEG - 2, 0, top)
    out_copy(NSEG - 2).start()
    v1, i1, v2, i2 = post(NSEG - 1, 1, top)
    out_copy(NSEG - 1).start()

    m1 = jnp.max(v1, axis=0, keepdims=True)
    i1v = jnp.min(jnp.where(v1 == m1, i1, S), axis=0, keepdims=True)
    cv2 = jnp.where(i1 == i1v, v2, v1)
    ci2 = jnp.where(i1 == i1v, i2, i1)
    m2 = jnp.max(cv2, axis=0, keepdims=True)
    i2v = jnp.min(jnp.where(cv2 == m2, ci2, S), axis=0, keepdims=True)
    idx = (jnp.min(i1v), jnp.min(i2v))
    rsel = (m1[:, 0:1], m2[:, 0:1])

    sb = modb[0:1, 3 * D:4 * D]
    cb = modb[0:1, 4 * D:5 * D]
    gb = modb[0:1, 5 * D:6 * D]
    brow = lax.broadcasted_iota(jnp.int32, (16, D), 0)
    blks, x1s, h2s, sel = [], [], [], []
    for j in range(2):
        b = pl.ds(pl.multiple_of((idx[j] // 16) * 16, 16), 16)
        x1 = x1b[b, :].astype(F32)
        h2 = _ln(x1) * (1.0 + cb) + sb
        blks.append(b)
        x1s.append(x1)
        h2s.append(h2)
        sel.append(jnp.sum(jnp.where(brow == idx[j] % 16, h2, 0.0), axis=0, keepdims=True))
    xs = jnp.concatenate(sel + [jnp.zeros((6, D), F32)], axis=0)

    pltpu.make_async_copy(wg, wg, sem_w.at[4]).wait()
    pltpu.make_async_copy(wu, wu, sem_w.at[5]).wait()
    wg32, wu32, wd32 = wg.bitcast(U32), wu.bitcast(U32), wd.bitcast(U32)
    npf = FF // 128
    gs = _panel_dot(xs, wg32, range(npf))
    us = _panel_dot(xs, wu32, range(npf))
    act = jnp.concatenate([g * jax.nn.sigmoid(g) * u for g, u in zip(gs, us)], axis=1)
    pltpu.make_async_copy(wd, wd, sem_w.at[6]).wait()
    y = jnp.concatenate(_panel_dot(act, wd32, range(KT)), axis=1)
    upd = [y[j:j + 1] * jax.nn.sigmoid(rsel[j]) for j in range(2)]

    pltpu.make_async_copy(ob, out_hbm, sem_o).wait()
    for j in range(2):
        base = (idx[j] // 16) * 16
        u = (jnp.where(brow + base == idx[0], upd[0], 0.0)
             + jnp.where(brow + base == idx[1], upd[1], 0.0))
        ob[blks[j], :] = (x1s[j] + gb * (h2s[j] + u)).astype(BF16)
        cp = pltpu.make_async_copy(ob.at[blks[j], :], out_hbm.at[blks[j], :], sem_p)
        cp.start()
        cp.wait()


@functools.partial(jax.jit, static_argnames=("A_seg_len",))
def pallas_adaLN_cond__memory_aug_recurrent_mem_tr__moe_arch_mod__prompt_kernel(
    A_x, A_mem0, A_Wq, A_Wk, A_Wv, A_Wo, A_seg_len, B_x, B_w_r, B_w_gate, B_w_up,
    B_w_down, c, w_mod,
):
    assert A_seg_len == SEG and A_x.shape == (1, S, D)
    assert A_Wq.shape == (D, NH, DH) and A_mem0.shape == (1, MM, D)
    del B_x
    hbm = pl.BlockSpec(memory_space=pl.ANY)
    vm = pl.BlockSpec(memory_space=pltpu.VMEM)
    npf = FF // 128
    out = pl.pallas_call(
        _kernel,
        out_shape=jax.ShapeDtypeStruct((S, D), BF16),
        in_specs=[hbm, hbm, vm, hbm, hbm, hbm, hbm, vm, hbm, hbm, hbm, vm, hbm],
        out_specs=hbm,
        scratch_shapes=[
            pltpu.VMEM((D // 16, 16 * NH, DH), BF16),
            pltpu.VMEM((D // 16, 16 * NH, DH), BF16),
            pltpu.VMEM((D // 16, 16 * NH, DH), BF16),
            pltpu.VMEM((NH, D // 2, 128), U32),
            pltpu.VMEM((NH, D // 2, 128), U32),
            pltpu.VMEM((NH, D // 2, 128), U32),
            pltpu.VMEM((KT, NH * DH, 128), BF16),
            pltpu.VMEM((npf, D, 128), BF16),
            pltpu.VMEM((npf, D, 128), BF16),
            pltpu.VMEM((KT, FF, 128), BF16),
            pltpu.VMEM((48, D, 128), BF16),
            pltpu.VMEM((S, D), BF16),
            pltpu.VMEM((NSEG, PR, D), BF16),
            pltpu.VMEM((NSEG * PR, D), F32),
            pltpu.VMEM((S, D), BF16),
            pltpu.VMEM((S, D), BF16),
            pltpu.VMEM((8, 6 * D), F32),
            pltpu.VMEM((MM, D), F32),
            pltpu.VMEM((SEG, D), F32),
            pltpu.VMEM((2, SEG, D), F32),
            pltpu.VMEM((L, NH * DH), F32),
            pltpu.SemaphoreType.DMA((3,)),
            pltpu.SemaphoreType.DMA((9,)),
            pltpu.SemaphoreType.DMA,
            pltpu.SemaphoreType.DMA,
        ],
        compiler_params=pltpu.CompilerParams(vmem_limit_bytes=120 * 2**20),
    )(
        A_x.reshape(S, D), A_x.reshape(NSEG, SEG, D), A_mem0.reshape(MM, D),
        A_Wq.reshape(D // 16, 16 * NH, DH), A_Wk.reshape(D // 16, 16 * NH, DH),
        A_Wv.reshape(D // 16, 16 * NH, DH), A_Wo.reshape(NH * DH, D),
        B_w_r.reshape(1, D), B_w_gate, B_w_up, B_w_down, c, w_mod,
    )
    return out.reshape(1, S, D)
```

```python
import functools

import jax
import jax.numpy as jnp
from jax import lax
import jax.experimental.pallas as pl
import jax.experimental.pallas.tpu as pltpu

F32 = jnp.float32
BF16 = jnp.bfloat16
U32 = jnp.uint32

S, D = 2048, 1024
NH, DH = 32, 128
MM, SEG = 8, 32
L = MM + SEG
LP = 48
NSEG = S // SEG
FF = 3584
KT = D // 128
EPS = 1e-05
LAG = 3
U = 2
PR = 8
XE = 8 * SEG


def _ln(x):
    m = jnp.mean(x, axis=-1, keepdims=True)
    xc = x - m
    v = jnp.mean(xc * xc, axis=-1, keepdims=True)
    return xc * lax.rsqrt(v + EPS)


def _rb(x):
    return x.astype(BF16).astype(F32)


def _w(ref32, j):
    return pltpu.bitcast(ref32[j], BF16)


def _panel_dot(lhs, ref32, panels):
    return [jnp.dot(lhs, _w(ref32, j), preferred_element_type=F32) for j in panels]


def _kernel(x_hbm, x3_hbm, mem0_ref, wq_hbm, wk_hbm, wv_hbm, wo_hbm, wr_ref, wg_hbm, wu_hbm,
            wd_hbm, c_ref, wmod_hbm, out_hbm,
            stg0, stg1, stg2, wq, wk, wv, wo, wg, wu, wd, wmod, xb, xpre, hpre, x1b, ob, modb,
            memb, hxb, oxb, obuf, sem_st, sem_w, sem_o, sem_p):
    def panel_copies(src, dst, panels, sem, col0=0):
        return [pltpu.make_async_copy(src.at[:, pl.ds((col0 + j) * 128, 128)],
                                      dst.at[col0 + j], sem) for j in range(panels)]

    cp_moda = panel_copies(wmod_hbm, wmod, 16, sem_w.at[0])
    cp_x0 = pltpu.make_async_copy(x_hbm.at[0:XE], xb.at[0:XE], sem_w.at[1])
    cp_x1 = pltpu.make_async_copy(x_hbm.at[XE:S], xb.at[XE:S], sem_w.at[7])
    cp_xp = pltpu.make_async_copy(x3_hbm.at[:, 0:PR, :], xpre, sem_w.at[8])
    cp_q = pltpu.make_async_copy(wq_hbm, stg0, sem_st.at[0])
    cp_k = pltpu.make_async_copy(wk_hbm, stg1, sem_st.at[1])
    cp_v = pltpu.make_async_copy(wv_hbm, stg2, sem_st.at[2])
    cp_wo = panel_copies(wo_hbm, wo, 8, sem_w.at[2])

    def panel_copy(src, dst, j, sem):
        return pltpu.make_async_copy(
            src.at[:, pl.ds(pl.multiple_of(j * 128, 128), 128)], dst.at[j], sem)

    def modb_copy(j):
        return panel_copy(wmod_hbm, wmod, 16 + j, sem_w.at[3])

    for cp in cp_moda:
        cp.start()
    cp_xp.start()
    cp_q.start()

    cv = c_ref[...].astype(F32)
    sc = jnp.broadcast_to(cv * jax.nn.sigmoid(cv), (8, D))
    wmod32 = wmod.bitcast(U32)

    def mod_part(lo, hi):
        for j in range(lo, hi):
            modb[:, (j // 8) * D + (j % 8) * 128:(j // 8) * D + (j % 8 + 1) * 128] = _rb(
                jnp.dot(sc, _w(wmod32, j), preferred_element_type=F32))

    def sa_ca():
        return modb[0:1, 0:D], modb[0:1, D:2 * D]

    for cp in cp_moda:
        cp.wait()
    mod_part(0, 16)
    modb[:, 2 * D:6 * D] = jnp.zeros((8, 4 * D), F32)
    memb[...] = mem0_ref[...].astype(F32)
    oxb[...] = jnp.zeros(oxb.shape, F32)
    cp_xp.wait()

    def pre_ln(i, carry):
        sa, ca = sa_ca()
        xv = jnp.concatenate([xpre[i * 4 + j] for j in range(4)], axis=0).astype(F32)
        hpre[pl.ds(pl.multiple_of(i * 32, 32), 32), :] = _ln(xv) * (1.0 + ca) + sa
        return carry

    lax.fori_loop(0, NSEG // 4, pre_ln, 0)

    qpre = stg0.bitcast(F32)

    def relayout(stg, dst, half=None):
        s32 = stg.bitcast(U32)

        def body(i, carry):
            if half is not None:
                qpre[2 * i + half] = jnp.dot(
                    hpre[half * 256:(half + 1) * 256, :], _w(wq, i),
                    preferred_element_type=F32)
            if half == 1:
                modb_copy(i).start()
            for b in range(2):
                blk = 2 * i + b
                r = pl.ds(pl.multiple_of(blk * 8, 8), 8)
                for p in range(NH // 2):
                    a = s32[blk, pl.ds(p, 8, stride=32), :]
                    b_ = s32[blk, pl.ds(16 + p, 8, stride=32), :]
                    dst[2 * p, r, :] = (a & 0xFFFF) | (b_ << 16)
                    dst[2 * p + 1, r, :] = (a >> 16) | ((b_ >> 16) << 16)
            return carry

        lax.fori_loop(0, D // 32, body, 0, unroll=2)

    cp_q.wait()
    cp_k.start()
    relayout(stg0, wq)
    cp_v.start()
    cp_k.wait()
    cp_x0.start()
    for cp in cp_wo:
        cp.start()
    relayout(stg1, wk, 0)
    cp_v.wait()
    relayout(stg2, wv, 1)
    cp_x1.start()

    def make_hx(s):
        r = pl.ds(pl.multiple_of(s * SEG, SEG), SEG)
        sa, ca = sa_ca()
        hxb[...] = _ln(xb[r, :].astype(F32)) * (1.0 + ca) + sa

    cp_x0.wait()
    make_hx(0)
    for cp in cp_wo:
        cp.wait()

    wo32 = wo.bitcast(U32)
    wr = wr_ref[...].astype(F32)

    row = lax.broadcasted_iota(jnp.int32, (L, LP), 0)
    col = lax.broadcasted_iota(jnp.int32, (L, LP), 1)
    amask = ((row < MM) & (col < L)) | (row >= col)
    scale = float(DH) ** (-0.5)

    trow = lax.broadcasted_iota(jnp.int32, (8, 128), 0)

    def post(s, slot, top, valid=None):
        r = pl.ds(pl.multiple_of(s * SEG, SEG), SEG)
        ga = modb[0:1, 2 * D:3 * D]
        sb = modb[0:1, 3 * D:4 * D]
        cb = modb[0:1, 4 * D:5 * D]
        gb = modb[0:1, 5 * D:6 * D]
        x1 = (xb[r, :].astype(F32) + ga * _rb(oxb[slot])).astype(BF16)
        x1b[r, :] = x1
        x1 = x1.astype(F32)
        h2 = _ln(x1) * (1.0 + cb) + sb
        ob[r, :] = (x1 + gb * h2).astype(BF16)
        rr = jnp.broadcast_to(jnp.sum(h2 * wr, axis=-1, keepdims=True), (SEG, 128))
        if valid is not None:
            rr = jnp.where(valid, rr, -jnp.inf)
        v1, i1, v2, i2 = top
        for j in range(SEG // 8):
            val = rr[j * 8:(j + 1) * 8]
            ix = trow + (s * SEG + j * 8)
            g1, g2 = val > v1, val > v2
            v2 = jnp.where(g1, v1, jnp.where(g2, val, v2))
            i2 = jnp.where(g1, i1, jnp.where(g2, ix, i2))
            v1 = jnp.where(g1, val, v1)
            i1 = jnp.where(g1, ix, i1)
        return v1, i1, v2, i2

    def out_copy(s):
        r = pl.ds(pl.multiple_of(s * SEG, SEG), SEG)
        return pltpu.make_async_copy(ob.at[r, :], out_hbm.at[r, :], sem_o)

    def group(g, top):
        s0 = U * g

        @pl.when(g == 1)
        def _():
            pltpu.make_async_copy(wmod.at[16:48], wmod.at[16:48], sem_w.at[3]).wait()
            mod_part(16, 48)

        @pl.when(g < FF // 128 // U)
        def _():
            for j in range(U):
                panel_copy(wg_hbm, wg, s0 + j, sem_w.at[4]).start()
                panel_copy(wu_hbm, wu, s0 + j, sem_w.at[5]).start()

        @pl.when(g < KT // U)
        def _():
            for j in range(U):
                panel_copy(wd_hbm, wd, s0 + j, sem_w.at[6]).start()

        @pl.when(g == (XE // SEG - 1) // U)
        def _():
            cp_x1.wait()

        @pl.when(g >= 2)
        def _():
            for j in range(U):
                out_copy(s0 - 2 * U + j).start()

        for j in range(U):
            top = step(s0 + j, j, top)
        return top

    def step(s, slot, top):
        top = post(jnp.maximum(s - U, 0), slot, top, s >= U)
        hq = jnp.concatenate([memb[...], hxb[PR:SEG, :]], axis=0)
        qrow = pl.ds(pl.multiple_of((s % 32) * PR, PR), PR)
        hh = jnp.concatenate([memb[...], hxb[...]], axis=0)
        zpad = jnp.zeros((LP - L, DH), F32)
        qs, ks, vs, ps = {}, {}, {}, {}

        def proj(h):
            q, = _panel_dot(hq, wq, (h,))
            k, = _panel_dot(hh, wk, (h,))
            v, = _panel_dot(hh, wv, (h,))
            qs[h] = jnp.concatenate([q[0:MM], qpre[2 * h + s // 32, qrow, :], q[MM:]], axis=0)
            ks[h] = jnp.concatenate([k, zpad], axis=0).astype(BF16)
            vs[h] = jnp.concatenate([v, zpad], axis=0).astype(BF16)

        def scores(h):
            sc_ = lax.dot_general(qs.pop(h), ks.pop(h), (((1,), (1,)), ((), ())),
                                  preferred_element_type=F32)
            sc_ = jnp.where(amask, sc_ * scale, -1000000000.0)
            e = jnp.exp(sc_ - jnp.max(sc_, axis=-1, keepdims=True))
            ps[h] = e / jnp.sum(e, axis=-1, keepdims=True)

        def pv(h):
            obuf[:, h * DH:(h + 1) * DH] = jnp.dot(ps.pop(h), vs.pop(h),
                                                   preferred_element_type=F32)

        HK = NH * DH // 2
        part = {}

        def oproj(n, half):
            w = pltpu.bitcast(wo32[n, half * (HK // 2):(half + 1) * (HK // 2), :], BF16)
            y = jnp.dot(obuf[:, half * HK:(half + 1) * HK], w, preferred_element_type=F32)
            if half == 0:
                part[n] = y
            else:
                y = y + part.pop(n)
                memb[:, n * 128:(n + 1) * 128] = y[0:MM]
                oxb[slot, :, n * 128:(n + 1) * 128] = y[MM:L]

        for i in range(NH + LAG):
            if i < NH:
                proj(i)
            else:
                if i == NH:
                    make_hx(jnp.minimum(s + 1, NSEG - 1))
                per = KT // LAG
                for n in range((i - NH) * per, KT if i == NH + LAG - 1 else (i - NH + 1) * per):
                    oproj(n, 0)
            if 0 <= i - 1 < NH:
                scores(i - 1)
            if 0 <= i - LAG < NH:
                pv(i - LAG)
        for n in range(KT):
            oproj(n, 1)

        return top

    ninf = jnp.full((8, 128), -jnp.inf, F32)
    top = lax.fori_loop(0, NSEG // U, group, (ninf, trow, ninf, trow + 8))
    for j in range(U):
        out_copy(NSEG - 2 * U + j).start()
    for j in range(U):
        top = post(NSEG - U + j, j, top)
        out_copy(NSEG - U + j).start()
    v1, i1, v2, i2 = top

    m1 = jnp.max(v1, axis=0, keepdims=True)
    i1v = jnp.min(jnp.where(v1 == m1, i1, S), axis=0, keepdims=True)
    cv2 = jnp.where(i1 == i1v, v2, v1)
    ci2 = jnp.where(i1 == i1v, i2, i1)
    m2 = jnp.max(cv2, axis=0, keepdims=True)
    i2v = jnp.min(jnp.where(cv2 == m2, ci2, S), axis=0, keepdims=True)
    idx = (jnp.min(i1v), jnp.min(i2v))
    rsel = (m1[:, 0:1], m2[:, 0:1])

    sb = modb[0:1, 3 * D:4 * D]
    cb = modb[0:1, 4 * D:5 * D]
    gb = modb[0:1, 5 * D:6 * D]
    brow = lax.broadcasted_iota(jnp.int32, (16, D), 0)
    blks, x1s, h2s, sel = [], [], [], []
    for j in range(2):
        b = pl.ds(pl.multiple_of((idx[j] // 16) * 16, 16), 16)
        x1 = x1b[b, :].astype(F32)
        h2 = _ln(x1) * (1.0 + cb) + sb
        blks.append(b)
        x1s.append(x1)
        h2s.append(h2)
        sel.append(jnp.sum(jnp.where(brow == idx[j] % 16, h2, 0.0), axis=0, keepdims=True))
    xs = jnp.concatenate(sel + [jnp.zeros((6, D), F32)], axis=0)

    pltpu.make_async_copy(wg, wg, sem_w.at[4]).wait()
    pltpu.make_async_copy(wu, wu, sem_w.at[5]).wait()
    wg32, wu32, wd32 = wg.bitcast(U32), wu.bitcast(U32), wd.bitcast(U32)
    npf = FF // 128
    gs = _panel_dot(xs, wg32, range(npf))
    us = _panel_dot(xs, wu32, range(npf))
    act = jnp.concatenate([g * jax.nn.sigmoid(g) * u for g, u in zip(gs, us)], axis=1)
    pltpu.make_async_copy(wd, wd, sem_w.at[6]).wait()
    y = jnp.concatenate(_panel_dot(act, wd32, range(KT)), axis=1)
    upd = [y[j:j + 1] * jax.nn.sigmoid(rsel[j]) for j in range(2)]

    pltpu.make_async_copy(ob, out_hbm, sem_o).wait()
    for j in range(2):
        base = (idx[j] // 16) * 16
        u = (jnp.where(brow + base == idx[0], upd[0], 0.0)
             + jnp.where(brow + base == idx[1], upd[1], 0.0))
        ob[blks[j], :] = (x1s[j] + gb * (h2s[j] + u)).astype(BF16)
        cp = pltpu.make_async_copy(ob.at[blks[j], :], out_hbm.at[blks[j], :], sem_p)
        cp.start()
        cp.wait()


@functools.partial(jax.jit, static_argnames=("A_seg_len",))
def pallas_adaLN_cond__memory_aug_recurrent_mem_tr__moe_arch_mod__prompt_kernel(
    A_x, A_mem0, A_Wq, A_Wk, A_Wv, A_Wo, A_seg_len, B_x, B_w_r, B_w_gate, B_w_up,
    B_w_down, c, w_mod,
):
    assert A_seg_len == SEG and A_x.shape == (1, S, D)
    assert A_Wq.shape == (D, NH, DH) and A_mem0.shape == (1, MM, D)
    del B_x
    hbm = pl.BlockSpec(memory_space=pl.ANY)
    vm = pl.BlockSpec(memory_space=pltpu.VMEM)
    npf = FF // 128
    out = pl.pallas_call(
        _kernel,
        out_shape=jax.ShapeDtypeStruct((S, D), BF16),
        in_specs=[hbm, hbm, vm, hbm, hbm, hbm, hbm, vm, hbm, hbm, hbm, vm, hbm],
        out_specs=hbm,
        scratch_shapes=[
            pltpu.VMEM((D // 16, 16 * NH, DH), BF16),
            pltpu.VMEM((D // 16, 16 * NH, DH), BF16),
            pltpu.VMEM((D // 16, 16 * NH, DH), BF16),
            pltpu.VMEM((NH, D // 2, 128), U32),
            pltpu.VMEM((NH, D // 2, 128), U32),
            pltpu.VMEM((NH, D // 2, 128), U32),
            pltpu.VMEM((KT, NH * DH, 128), BF16),
            pltpu.VMEM((npf, D, 128), BF16),
            pltpu.VMEM((npf, D, 128), BF16),
            pltpu.VMEM((KT, FF, 128), BF16),
            pltpu.VMEM((48, D, 128), BF16),
            pltpu.VMEM((S, D), BF16),
            pltpu.VMEM((NSEG, PR, D), BF16),
            pltpu.VMEM((NSEG * PR, D), F32),
            pltpu.VMEM((S, D), BF16),
            pltpu.VMEM((S, D), BF16),
            pltpu.VMEM((8, 6 * D), F32),
            pltpu.VMEM((MM, D), F32),
            pltpu.VMEM((SEG, D), F32),
            pltpu.VMEM((U, SEG, D), F32),
            pltpu.VMEM((L, NH * DH), F32),
            pltpu.SemaphoreType.DMA((3,)),
            pltpu.SemaphoreType.DMA((9,)),
            pltpu.SemaphoreType.DMA,
            pltpu.SemaphoreType.DMA,
        ],
        compiler_params=pltpu.CompilerParams(vmem_limit_bytes=120 * 2**20),
    )(
        A_x.reshape(S, D), A_x.reshape(NSEG, SEG, D), A_mem0.reshape(MM, D),
        A_Wq.reshape(D // 16, 16 * NH, DH), A_Wk.reshape(D // 16, 16 * NH, DH),
        A_Wv.reshape(D // 16, 16 * NH, DH), A_Wo.reshape(NH * DH, D),
        B_w_r.reshape(1, D), B_w_gate, B_w_up, B_w_down, c, w_mod,
    )
    return out.reshape(1, S, D)
```

```python
import functools

import jax
import jax.numpy as jnp
from jax import lax
import jax.experimental.pallas as pl
import jax.experimental.pallas.tpu as pltpu

F32 = jnp.float32
BF16 = jnp.bfloat16
U32 = jnp.uint32

S, D = 2048, 1024
NH, DH = 32, 128
MM, SEG = 8, 32
L = MM + SEG
LP = 48
NSEG = S // SEG
FF = 3584
KT = D // 128
EPS = 1e-05
LAG = 3
U = 2
PR = 8
XE = 8 * SEG


def _ln(x):
    m = jnp.mean(x, axis=-1, keepdims=True)
    xc = x - m
    v = jnp.mean(xc * xc, axis=-1, keepdims=True)
    return xc * lax.rsqrt(v + EPS)


def _rb(x):
    return x.astype(BF16).astype(F32)


def _w(ref32, j):
    return pltpu.bitcast(ref32[j], BF16)


def _panel_dot(lhs, ref32, panels):
    return [jnp.dot(lhs, _w(ref32, j), preferred_element_type=F32) for j in panels]


def _kernel(x_hbm, x3_hbm, mem0_ref, wq_hbm, wk_hbm, wv_hbm, wo_hbm, wr_ref, wg_hbm, wu_hbm,
            wd_hbm, c_ref, wmod_hbm, out_hbm,
            stg0, stg1, stg2, wq, wk, wv, wo, wg, wu, wd, wmod, xb, xpre, hpre, x1b, ob, modb,
            memb, hxb, oxb, obuf, sem_st, sem_w, sem_o, sem_p):
    def panel_copies(src, dst, panels, sem, col0=0):
        return [pltpu.make_async_copy(src.at[:, pl.ds((col0 + j) * 128, 128)],
                                      dst.at[col0 + j], sem) for j in range(panels)]

    cp_moda = panel_copies(wmod_hbm, wmod, 16, sem_w.at[0])
    cp_x0 = pltpu.make_async_copy(x_hbm.at[0:XE], xb.at[0:XE], sem_w.at[1])
    cp_x1 = pltpu.make_async_copy(x_hbm.at[XE:S], xb.at[XE:S], sem_w.at[7])
    cp_xp = pltpu.make_async_copy(x3_hbm.at[:, 0:PR, :], xpre, sem_w.at[8])
    cp_q = pltpu.make_async_copy(wq_hbm, stg0, sem_st.at[0])
    cp_k = pltpu.make_async_copy(wk_hbm, stg1, sem_st.at[1])
    cp_v = pltpu.make_async_copy(wv_hbm, stg2, sem_st.at[2])
    cp_wo = panel_copies(wo_hbm, wo, 8, sem_w.at[2])

    def panel_copy(src, dst, j, sem):
        return pltpu.make_async_copy(
            src.at[:, pl.ds(pl.multiple_of(j * 128, 128), 128)], dst.at[j], sem)

    def modb_copy(j):
        return panel_copy(wmod_hbm, wmod, 16 + j, sem_w.at[3])

    for cp in cp_moda:
        cp.start()
    cp_xp.start()
    cp_q.start()

    cv = c_ref[...].astype(F32)
    sc = jnp.broadcast_to(cv * jax.nn.sigmoid(cv), (8, D))
    wmod32 = wmod.bitcast(U32)

    def mod_part(lo, hi):
        for j in range(lo, hi):
            modb[:, (j // 8) * D + (j % 8) * 128:(j // 8) * D + (j % 8 + 1) * 128] = _rb(
                jnp.dot(sc, _w(wmod32, j), preferred_element_type=F32))

    def sa_ca():
        return modb[0:1, 0:D], modb[0:1, D:2 * D]

    for cp in cp_moda:
        cp.wait()
    mod_part(0, 16)
    modb[:, 2 * D:6 * D] = jnp.zeros((8, 4 * D), F32)
    memb[...] = mem0_ref[...].astype(F32)
    oxb[...] = jnp.zeros(oxb.shape, F32)
    cp_xp.wait()

    def pre_ln(i, carry):
        sa, ca = sa_ca()
        xv = jnp.concatenate([xpre[i * 4 + j] for j in range(4)], axis=0).astype(F32)
        hpre[pl.ds(pl.multiple_of(i * 32, 32), 32), :] = _ln(xv) * (1.0 + ca) + sa
        return carry

    lax.fori_loop(0, NSEG // 4, pre_ln, 0)

    qpre = stg0.bitcast(F32)

    def relayout(stg, dst, half=None):
        s32 = stg.bitcast(U32)

        def body(i, carry):
            if half is not None:
                qpre[2 * i + half] = jnp.dot(
                    hpre[half * 256:(half + 1) * 256, :], _w(wq, i),
                    preferred_element_type=F32)
            if half == 1:
                modb_copy(i).start()
            for b in range(2):
                blk = 2 * i + b
                r = pl.ds(pl.multiple_of(blk * 8, 8), 8)
                for p in range(NH // 2):
                    a = s32[blk, pl.ds(p, 8, stride=32), :]
                    b_ = s32[blk, pl.ds(16 + p, 8, stride=32), :]
                    dst[2 * p, r, :] = (a & 0xFFFF) | (b_ << 16)
                    dst[2 * p + 1, r, :] = (a >> 16) | ((b_ >> 16) << 16)
            return carry

        lax.fori_loop(0, D // 32, body, 0, unroll=2)

    cp_q.wait()
    cp_k.start()
    relayout(stg0, wq)
    cp_v.start()
    cp_k.wait()
    cp_x0.start()
    for cp in cp_wo:
        cp.start()
    relayout(stg1, wk, 0)
    cp_v.wait()
    relayout(stg2, wv, 1)
    cp_x1.start()

    def make_hx(s):
        r = pl.ds(pl.multiple_of(s * SEG, SEG), SEG)
        sa, ca = sa_ca()
        hxb[...] = _ln(xb[r, :].astype(F32)) * (1.0 + ca) + sa

    cp_x0.wait()
    make_hx(0)
    for cp in cp_wo:
        cp.wait()

    wo32 = wo.bitcast(U32)
    wr = wr_ref[...].astype(F32).reshape(1, D)

    row = lax.broadcasted_iota(jnp.int32, (L, LP), 0)
    col = lax.broadcasted_iota(jnp.int32, (L, LP), 1)
    amask = ((row < MM) & (col < L)) | (row >= col)
    scale = float(DH) ** (-0.5)

    trow = lax.broadcasted_iota(jnp.int32, (8, 128), 0)

    def post(s, slot, top, valid=None):
        r = pl.ds(pl.multiple_of(s * SEG, SEG), SEG)
        ga = modb[0:1, 2 * D:3 * D]
        sb = modb[0:1, 3 * D:4 * D]
        cb = modb[0:1, 4 * D:5 * D]
        gb = modb[0:1, 5 * D:6 * D]
        x1 = (xb[r, :].astype(F32) + ga * _rb(oxb[slot])).astype(BF16)
        x1b[r, :] = x1
        x1 = x1.astype(F32)
        h2 = _ln(x1) * (1.0 + cb) + sb
        ob[r, :] = (x1 + gb * h2).astype(BF16)
        rr = jnp.broadcast_to(jnp.sum(h2 * wr, axis=-1, keepdims=True), (SEG, 128))
        if valid is not None:
            rr = jnp.where(valid, rr, -jnp.inf)
        v1, i1, v2, i2 = top
        for j in range(SEG // 8):
            val = rr[j * 8:(j + 1) * 8]
            ix = trow + (s * SEG + j * 8)
            g1, g2 = val > v1, val > v2
            v2 = jnp.where(g1, v1, jnp.where(g2, val, v2))
            i2 = jnp.where(g1, i1, jnp.where(g2, ix, i2))
            v1 = jnp.where(g1, val, v1)
            i1 = jnp.where(g1, ix, i1)
        return v1, i1, v2, i2

    def out_copy(s):
        r = pl.ds(pl.multiple_of(s * SEG, SEG), SEG)
        return pltpu.make_async_copy(ob.at[r, :], out_hbm.at[r, :], sem_o)

    def group(g, top):
        s0 = U * g

        @pl.when(g == 1)
        def _():
            pltpu.make_async_copy(wmod.at[16:48], wmod.at[16:48], sem_w.at[3]).wait()
            mod_part(16, 48)

        @pl.when(g < FF // 128 // U)
        def _():
            for j in range(U):
                panel_copy(wg_hbm, wg, s0 + j, sem_w.at[4]).start()
                panel_copy(wu_hbm, wu, s0 + j, sem_w.at[5]).start()

        @pl.when(g < KT // U)
        def _():
            for j in range(U):
                panel_copy(wd_hbm, wd, s0 + j, sem_w.at[6]).start()

        @pl.when(g == (XE // SEG - 1) // U)
        def _():
            cp_x1.wait()

        @pl.when(g >= 2)
        def _():
            for j in range(U):
                out_copy(s0 - 2 * U + j).start()

        for j in range(U):
            top = step(s0 + j, j, top)
        return top

    def step(s, slot, top):
        top = post(jnp.maximum(s - U, 0), slot, top, s >= U)
        hq = jnp.concatenate([memb[...], hxb[PR:SEG, :]], axis=0)
        qrow = pl.ds(pl.multiple_of((s % 32) * PR, PR), PR)
        hh = jnp.concatenate([memb[...], hxb[...]], axis=0)
        zpad = jnp.zeros((LP - L, DH), F32)
        qs, ks, vs, ps = {}, {}, {}, {}

        def proj(h):
            q, = _panel_dot(hq, wq, (h,))
            k, = _panel_dot(hh, wk, (h,))
            v, = _panel_dot(hh, wv, (h,))
            qs[h] = jnp.concatenate([q[0:MM], qpre[2 * h + s // 32, qrow, :], q[MM:]], axis=0)
            ks[h] = jnp.concatenate([k, zpad], axis=0).astype(BF16)
            vs[h] = jnp.concatenate([v, zpad], axis=0).astype(BF16)

        def scores(h):
            sc_ = lax.dot_general(qs.pop(h), ks.pop(h), (((1,), (1,)), ((), ())),
                                  preferred_element_type=F32)
            sc_ = jnp.where(amask, sc_ * scale, -1000000000.0)
            e = jnp.exp(sc_ - jnp.max(sc_, axis=-1, keepdims=True))
            ps[h] = e / jnp.sum(e, axis=-1, keepdims=True)

        def pv(h):
            obuf[:, h * DH:(h + 1) * DH] = jnp.dot(ps.pop(h), vs.pop(h),
                                                   preferred_element_type=F32)

        HK = NH * DH // 2
        part = {}

        def oproj(n, half):
            w = pltpu.bitcast(wo32[n, half * (HK // 2):(half + 1) * (HK // 2), :], BF16)
            y = jnp.dot(obuf[:, half * HK:(half + 1) * HK], w, preferred_element_type=F32)
            if half == 0:
                part[n] = y
            else:
                y = y + part.pop(n)
                memb[:, n * 128:(n + 1) * 128] = y[0:MM]
                oxb[slot, :, n * 128:(n + 1) * 128] = y[MM:L]

        for i in range(NH + LAG):
            if i < NH:
                proj(i)
            else:
                if i == NH:
                    make_hx(jnp.minimum(s + 1, NSEG - 1))
                per = KT // LAG
                for n in range((i - NH) * per, KT if i == NH + LAG - 1 else (i - NH + 1) * per):
                    oproj(n, 0)
            if 0 <= i - 1 < NH:
                scores(i - 1)
            if 0 <= i - LAG < NH:
                pv(i - LAG)
        for n in range(KT):
            oproj(n, 1)

        return top

    ninf = jnp.full((8, 128), -jnp.inf, F32)
    top = lax.fori_loop(0, NSEG // U, group, (ninf, trow, ninf, trow + 8))
    for j in range(U):
        out_copy(NSEG - 2 * U + j).start()
    for j in range(U):
        top = post(NSEG - U + j, j, top)
        out_copy(NSEG - U + j).start()
    v1, i1, v2, i2 = top

    m1 = jnp.max(v1, axis=0, keepdims=True)
    i1v = jnp.min(jnp.where(v1 == m1, i1, S), axis=0, keepdims=True)
    cv2 = jnp.where(i1 == i1v, v2, v1)
    ci2 = jnp.where(i1 == i1v, i2, i1)
    m2 = jnp.max(cv2, axis=0, keepdims=True)
    i2v = jnp.min(jnp.where(cv2 == m2, ci2, S), axis=0, keepdims=True)
    idx = (jnp.min(i1v), jnp.min(i2v))
    rsel = (m1[:, 0:1], m2[:, 0:1])

    sb = modb[0:1, 3 * D:4 * D]
    cb = modb[0:1, 4 * D:5 * D]
    gb = modb[0:1, 5 * D:6 * D]
    brow = lax.broadcasted_iota(jnp.int32, (16, D), 0)
    blks, x1s, h2s, sel = [], [], [], []
    for j in range(2):
        b = pl.ds(pl.multiple_of((idx[j] // 16) * 16, 16), 16)
        x1 = x1b[b, :].astype(F32)
        h2 = _ln(x1) * (1.0 + cb) + sb
        blks.append(b)
        x1s.append(x1)
        h2s.append(h2)
        sel.append(jnp.sum(jnp.where(brow == idx[j] % 16, h2, 0.0), axis=0, keepdims=True))
    xs = jnp.concatenate(sel + [jnp.zeros((6, D), F32)], axis=0)

    pltpu.make_async_copy(wg, wg, sem_w.at[4]).wait()
    pltpu.make_async_copy(wu, wu, sem_w.at[5]).wait()
    wg32, wu32, wd32 = wg.bitcast(U32), wu.bitcast(U32), wd.bitcast(U32)
    npf = FF // 128
    gs = _panel_dot(xs, wg32, range(npf))
    us = _panel_dot(xs, wu32, range(npf))
    act = jnp.concatenate([g * jax.nn.sigmoid(g) * u for g, u in zip(gs, us)], axis=1)
    pltpu.make_async_copy(wd, wd, sem_w.at[6]).wait()
    y = jnp.concatenate(_panel_dot(act, wd32, range(KT)), axis=1)
    upd = [y[j:j + 1] * jax.nn.sigmoid(rsel[j]) for j in range(2)]

    pltpu.make_async_copy(ob, out_hbm, sem_o).wait()
    for j in range(2):
        base = (idx[j] // 16) * 16
        u = (jnp.where(brow + base == idx[0], upd[0], 0.0)
             + jnp.where(brow + base == idx[1], upd[1], 0.0))
        ob[blks[j], :] = (x1s[j] + gb * (h2s[j] + u)).astype(BF16)
    patch = [pltpu.make_async_copy(ob.at[blks[j], :], out_hbm.at[blks[j], :], sem_p.at[j])
             for j in range(2)]
    patch[0].start()

    @pl.when(idx[0] // 16 != idx[1] // 16)
    def _():
        patch[1].start()
        patch[1].wait()

    patch[0].wait()


@functools.partial(jax.jit, static_argnames=("A_seg_len",))
def pallas_adaLN_cond__memory_aug_recurrent_mem_tr__moe_arch_mod__prompt_kernel(
    A_x, A_mem0, A_Wq, A_Wk, A_Wv, A_Wo, A_seg_len, B_x, B_w_r, B_w_gate, B_w_up,
    B_w_down, c, w_mod,
):
    assert A_seg_len == SEG and A_x.shape == (1, S, D)
    assert A_Wq.shape == (D, NH, DH) and A_mem0.shape == (1, MM, D)
    del B_x
    hbm = pl.BlockSpec(memory_space=pl.ANY)
    vm = pl.BlockSpec(memory_space=pltpu.VMEM)
    npf = FF // 128
    out = pl.pallas_call(
        _kernel,
        out_shape=jax.ShapeDtypeStruct((S, D), BF16),
        in_specs=[hbm, hbm, vm, hbm, hbm, hbm, hbm, vm, hbm, hbm, hbm, vm, hbm],
        out_specs=hbm,
        scratch_shapes=[
            pltpu.VMEM((D // 16, 16 * NH, DH), BF16),
            pltpu.VMEM((D // 16, 16 * NH, DH), BF16),
            pltpu.VMEM((D // 16, 16 * NH, DH), BF16),
            pltpu.VMEM((NH, D // 2, 128), U32),
            pltpu.VMEM((NH, D // 2, 128), U32),
            pltpu.VMEM((NH, D // 2, 128), U32),
            pltpu.VMEM((KT, NH * DH, 128), BF16),
            pltpu.VMEM((npf, D, 128), BF16),
            pltpu.VMEM((npf, D, 128), BF16),
            pltpu.VMEM((KT, FF, 128), BF16),
            pltpu.VMEM((48, D, 128), BF16),
            pltpu.VMEM((S, D), BF16),
            pltpu.VMEM((NSEG, PR, D), BF16),
            pltpu.VMEM((NSEG * PR, D), F32),
            pltpu.VMEM((S, D), BF16),
            pltpu.VMEM((S, D), BF16),
            pltpu.VMEM((8, 6 * D), F32),
            pltpu.VMEM((MM, D), F32),
            pltpu.VMEM((SEG, D), F32),
            pltpu.VMEM((U, SEG, D), F32),
            pltpu.VMEM((L, NH * DH), F32),
            pltpu.SemaphoreType.DMA((3,)),
            pltpu.SemaphoreType.DMA((9,)),
            pltpu.SemaphoreType.DMA,
            pltpu.SemaphoreType.DMA((2,)),
        ],
        compiler_params=pltpu.CompilerParams(vmem_limit_bytes=120 * 2**20),
    )(
        A_x.reshape(S, D), A_x.reshape(NSEG, SEG, D), A_mem0.reshape(MM, D),
        A_Wq.reshape(D // 16, 16 * NH, DH), A_Wk.reshape(D // 16, 16 * NH, DH),
        A_Wv.reshape(D // 16, 16 * NH, DH), A_Wo.reshape(NH * DH, D),
        B_w_r, B_w_gate, B_w_up, B_w_down, c, w_mod,
    )
    return out.reshape(1, S, D)
```
